```python
import jax
import jax.numpy as jnp

def _softmax(x, axis=-1):
    return jax.nn.softmax(x, axis=axis)
def _gelu(x):
    return jax.nn.gelu(x, approximate=True)
def _silu(x):
    return jax.nn.silu(x)
def _sigmoid(x):
    return jax.nn.sigmoid(x)
def _layernorm(x, axis=-1, eps=1e-5):
    m = jnp.mean(x, axis=axis, keepdims=True)
    v = jnp.var(x, axis=axis, keepdims=True)
    return (x - m) / jnp.sqrt(v + eps)
def _scatter_add(tgt, idx, src, axis=0):
    return tgt.at[idx].add(src)
def _segment_sum(src, seg, n):
    return jax.ops.segment_sum(src, seg, n)
class _Rng:
    def __init__(self, key):
        self._k = key
    def _next(self):
        self._k, sub = jax.random.split(self._k)
        return sub
    def normal(self, shape):
        return jax.random.normal(self._next(), shape, dtype=jnp.bfloat16)
    def randint(self, lo, hi, shape):
        return jax.random.randint(self._next(), shape, lo, hi, dtype=jnp.int32)
    def uniform(self, shape, lo=0.0, hi=1.0):
        return jax.random.uniform(self._next(), shape, jnp.bfloat16, lo, hi)
    def permutation(self, n):
        return jax.random.permutation(self._next(), n)


kernel_name = 'gated_mix__mha_block_cached__moe_arch_mod__decode'

def setup_inputs():
    _rng = _Rng(jax.random.key(int.from_bytes(__import__("os").urandom(4), "little")))
    _w = (lambda a: (lambda t: t.astype(jnp.bfloat16) if jnp.issubdtype(t.dtype, jnp.floating) else t)(jnp.asarray(a)))
    def _A_setup():
        B, Sq, D = 4, 1, 1024
        H, Sk, Dh = 32, 8192, 128
        return {
            "x": _w((lambda *s: _rng.normal(s) * 0.05)(B, Sq, D)),
            "k_cache": _w((lambda *s: _rng.normal(s) * 0.05)(B, H, Sk, Dh)),
            "v_cache": _w((lambda *s: _rng.normal(s) * 0.05)(B, H, Sk, Dh)),
            "wq": _w((lambda *s: _rng.normal(s) * 0.05)(D, H * Dh) * (D ** -0.5)),
            "wo": _w((lambda *s: _rng.normal(s) * 0.05)(H * Dh, D) * ((H * Dh) ** -0.5)),
        }
    _A_in = _A_setup()

    def _B_setup():
        B, S, D, F, C = 4, 1, 1024, 3584, 1
        return {
            "x": _w((lambda *s: _rng.normal(s) * 0.05)(B, S, D)),
            "w_r": _w((lambda *s: _rng.normal(s) * 0.05)(D)),
            "w_gate": _w((lambda *s: _rng.normal(s) * 0.05)(D, F)),
            "w_up": _w((lambda *s: _rng.normal(s) * 0.05)(D, F)),
            "w_down": _w((lambda *s: _rng.normal(s) * 0.05)(F, D)),
        }
    _B_in = _B_setup()

    return {
        "A_x": _A_in["x"],
        "A_k_cache": _A_in["k_cache"],
        "A_v_cache": _A_in["v_cache"],
        "A_wq": _A_in["wq"],
        "A_wo": _A_in["wo"],
        "B_x": _B_in["x"],
        "B_w_r": _B_in["w_r"],
        "B_w_gate": _B_in["w_gate"],
        "B_w_up": _B_in["w_up"],
        "B_w_down": _B_in["w_down"],
        "gate_w": _w((lambda *s: _rng.normal(s) * 0.05)(1024)),
    }

def reference(A_x, A_k_cache, A_v_cache, A_wq, A_wo, B_x, B_w_r, B_w_gate, B_w_up, B_w_down, gate_w):
    def _A_ref(x, k_cache, v_cache, wq, wo):
        B, Sq, D = x.shape
        H, Dh = 32, 128
        q = (lambda x, *d: x.transpose(*d))((x @ wq).reshape(B, Sq, H, Dh), 0, 2, 1, 3)
        scores = jnp.einsum("bhqd,bhkd->bhqk", q, k_cache) * (Dh ** -0.5)
        p = _softmax(scores, axis=-1)
        o = jnp.einsum("bhqk,bhkd->bhqd", p, v_cache)
        return (lambda x, *d: x.transpose(*d))(o, 0, 2, 1, 3).reshape(B, Sq, H * Dh) @ wo

    def _B_ref(x, w_r, w_gate, w_up, w_down):
        B, S, D = x.shape
        C = 1
        r = x @ w_r
        idx = jnp.argsort(-r, axis=-1)[:, :C]
        idx_e = jnp.repeat(idx.reshape(B, C, 1), D, axis=2)
        x_sel = jnp.take_along_axis(x, idx_e, axis=1)
        g = _silu(x_sel @ w_gate)
        u = x_sel @ w_up
        y = (g * u) @ w_down
        r_sel = _sigmoid(jnp.take_along_axis(r, idx, axis=1))
        y = y * r_sel.reshape(B, C, 1)
        b_off = (jnp.arange(B) * S).reshape(B, 1)
        flat_idx = (idx + b_off).reshape(B * C)
        zero = (x * 0.0).reshape(B * S, D)
        upd = _scatter_add(zero, flat_idx, y.reshape(B * C, D), axis=0)
        return x + upd.reshape(B, S, D)

    x = A_x
    g = _sigmoid((x * gate_w).sum(-1, keepdims=True))
    a = _A_ref(x, A_k_cache, A_v_cache, A_wq, A_wo)
    b = _B_ref(x, B_w_r, B_w_gate, B_w_up, B_w_down)
    return g * a + (1 - g) * b
```

```python
import functools

import jax
import jax.numpy as jnp
from jax import lax
import jax.experimental.pallas as pl
import jax.experimental.pallas.tpu as pltpu

F32, BF16 = jnp.float32, jnp.bfloat16

B, D, H, S, DH, F = 4, 1024, 32, 8192, 128, 3584
HG = 8
G = B * H // HG
SCALE = DH ** -0.5
R = 128
SEG = 16
NS = S // R
T = G * NS
L = 14
NB = L + 1
KB = D // 128
FB = F // 128


def _kernel(x_hbm, k_hbm, v_hbm, wq_hbm, wo_hbm, wr_hbm, wg_hbm, wu_hbm, wd_hbm, gw_hbm, o_ref,
            kv, wq_s, wo_s, wgu_s, wd_s, x_s, wr_s, gw_s, xb_s, q_s, o_s, g_s, u_s, sc_s, a_s,
            sem_kv, sem_w, sem_wd):
    def kv_copy(t, j, which):
        base = pl.multiple_of((t % NS) * R, R)
        sl = which * NB + t % NB
        src = (k_hbm, v_hbm)[which]
        pltpu.make_async_copy(src.at[t // NS, :, pl.ds(base + j * SEG, SEG)],
                              kv.at[sl, :, pl.ds(j * SEG, SEG)], sem_kv.at[sl]).start(priority=which)

    def kv_dmas(t):
        return [functools.partial(kv_copy, t, j, w) for j in range(R // SEG) for w in (0, 1)]

    def wd_copy(blk, j, which):
        b = blk + which * (FB // 2)
        r = pl.multiple_of(b * 128 + j * 16, 16)
        pltpu.make_async_copy(wd_hbm.at[pl.ds(r, 16)], wd_s.at[pl.ds(r, 16)], sem_wd.at[b]).start(priority=which)

    def wd_dmas(blk):
        return [functools.partial(wd_copy, blk, j, w) for j in range(8) for w in (0, 1)]

    def wait_all(ref, sem):
        pltpu.make_async_copy(ref, ref, sem).wait()

    small = [pltpu.make_async_copy(x_hbm, x_s, sem_w.at[4]),
             pltpu.make_async_copy(wr_hbm, wr_s, sem_w.at[5]),
             pltpu.make_async_copy(gw_hbm, gw_s, sem_w.at[6])]
    for c in small:
        c.start()

    def p1(r8, c):
        r = pl.multiple_of(r8 * 8, 8)
        for cb in range(F // 256):
            for w, src in enumerate((wg_hbm, wu_hbm)):
                pltpu.make_async_copy(src.at[:, pl.ds(r, 8), pl.ds(cb * 256, 256)],
                                      wgu_s.at[w, :, pl.ds(r, 8), pl.ds(cb * 256, 256)],
                                      sem_w.at[w]).start(priority=w)
        return c
    lax.fori_loop(0, 16, p1, 0)

    for c in small:
        c.wait()
    x4 = x_s[...].astype(F32)
    x8 = jnp.concatenate([x4, jnp.zeros_like(x4)], axis=0)
    for kb in range(KB):
        xb_s[kb] = x8[:, kb * 128:(kb + 1) * 128]
    gate = jax.nn.sigmoid(jnp.sum(x8 * gw_s[...].astype(F32).reshape(1, D), axis=-1, keepdims=True))
    rsel = jax.nn.sigmoid(jnp.sum(x8 * wr_s[...].astype(F32).reshape(1, D), axis=-1, keepdims=True))
    sc_s[0] = jnp.broadcast_to(gate, (8, 128))
    sc_s[1] = jnp.broadcast_to(rsel, (8, 128))
    q_s[...] = jnp.zeros_like(q_s)
    g_s[...] = jnp.zeros_like(g_s)
    u_s[...] = jnp.zeros_like(u_s)
    o_s[...] = jnp.zeros_like(o_s)
    a_s[...] = jnp.zeros_like(a_s)

    def p2_issue(r8):
        r = pl.multiple_of(r8 * 8, 8)
        for cb in range(16):
            pltpu.make_async_copy(wq_hbm.at[:, pl.ds(r, 8), pl.ds(cb * 256, 256)],
                                  wq_s.at[:, pl.ds(r, 8), pl.ds(cb * 256, 256)], sem_w.at[2]).start(priority=0)
            r0 = pl.multiple_of(r8 * 32 + (cb // 4) * 8, 8)
            c0 = (cb % 4) * 256
            pltpu.make_async_copy(wo_hbm.at[:, pl.ds(r0, 8), pl.ds(c0, 256)],
                                  wo_s.at[:, pl.ds(r0, 8), pl.ds(c0, 256)], sem_w.at[3]).start(priority=1)

    def acc_cols(dst, part):
        for j in range(part.shape[1] // 128):
            dst[j * 8:(j + 1) * 8, :] += part[:, j * 128:(j + 1) * 128]

    def p2a(r8, c):
        p2_issue(r8)
        return c
    lax.fori_loop(0, 8, p2a, 0)
    wait_all(wgu_s.at[0], sem_w.at[0])
    wait_all(wgu_s.at[1], sem_w.at[1])

    def p2b(r8, c):
        p2_issue(r8)
        kb = r8 - 8
        xk = xb_s[kb].astype(BF16)
        acc_cols(g_s, jnp.dot(xk, wgu_s[0, kb], preferred_element_type=F32))
        acc_cols(u_s, jnp.dot(xk, wgu_s[1, kb], preferred_element_type=F32))
        return c
    lax.fori_loop(8, 16, p2b, 0)

    def p3a(t, c):
        for d in kv_dmas(t):
            d()
        return c
    lax.fori_loop(0, L - KB, p3a, 0)
    gg = g_s[...]
    g_s[...] = gg * jax.nn.sigmoid(gg) * u_s[...]
    wait_all(wq_s, sem_w.at[2])

    def p3b(t, c):
        for d in kv_dmas(t):
            d()
        kb = t - (L - KB)
        acc_cols(q_s, jnp.dot(xb_s[kb].astype(BF16), wq_s[kb], preferred_element_type=F32))
        return c
    lax.fori_loop(L - KB, L, p3b, 0)

    neg = jnp.full((8, 128), -jnp.inf, F32)
    zero = jnp.zeros((8, 128), F32)
    row = lax.broadcasted_iota(jnp.int32, (8, R), 0)

    def finalize(g, l, acc):
        o_s[pl.ds(pl.multiple_of(g * 8, 8), 8), :] = acc / jnp.sum(l, axis=-1, keepdims=True)

    def step(t, carry, dmas, fin):
        m, l, acc = carry
        g = t // NS
        c = t % NS
        ks, vs = t % NB, NB + t % NB
        wait_all(kv.at[ks], sem_kv.at[ks])
        wait_all(kv.at[vs], sem_kv.at[vs])
        first = c == 0
        m = jnp.where(first, neg, m)
        l = jnp.where(first, zero, l)
        acc = jnp.where(first, zero, acc)
        q = q_s[pl.ds((g % 4) * 64 + g // 4, 8, stride=8), :].astype(BF16)
        s = None
        for j in range(HG):
            dmas[j]()
            sj = lax.dot_general(q, kv[ks, j], (((1,), (1,)), ((), ())), preferred_element_type=F32)
            s = sj if s is None else jnp.where(row == j, sj, s)
        s = s * SCALE
        m_new = jnp.maximum(m, jnp.max(s, axis=-1, keepdims=True))
        alpha = jnp.exp(m - m_new)
        p = jnp.exp(s - m_new)
        l = l * alpha + p
        pv = None
        for j in range(HG):
            dmas[HG + j]()
            pj = jnp.where(row == j, p, 0.0).astype(BF16)
            d = jnp.dot(pj, kv[vs, j], preferred_element_type=F32)
            pv = d if pv is None else pv + d
        acc = acc * alpha + pv
        if fin:
            @pl.when(c == NS - 1)
            def _():
                finalize(g, l, acc)
        return m_new, l, acc

    cr = lax.fori_loop(0, T - L, lambda t, cr: step(t, cr, kv_dmas(t + L), True), (neg, zero, zero))

    def wo_block(h):
        lhs = o_s[pl.ds(h, 8, stride=H), :].astype(BF16)
        w = wo_s[h // 4, pl.ds(pl.multiple_of((h % 4) * 128, 128), 128), :]
        return jnp.dot(lhs, w, preferred_element_type=F32)

    wait_all(wo_s, sem_w.at[3])

    def tail(it, cr, with_wo):
        cr = step(T - L + it, cr, wd_dmas(it), False)
        if with_wo:
            a_s[...] += wo_block(2 * it) + wo_block(2 * it + 1)
        return cr
    cr = lax.fori_loop(0, 12, lambda it, cr: tail(it, cr, True), cr)
    cr = lax.fori_loop(12, L, lambda it, cr: tail(it, cr, False), cr)
    finalize(G - 1, cr[1], cr[2])

    a = lax.fori_loop(H - HG, H, lambda h, acc: acc + wo_block(h), a_s[...])

    def down(b, acc):
        rows = pl.ds(pl.multiple_of(b * 128, 128), 128)
        wait_all(wd_s.at[rows], sem_wd.at[b])
        lhs = g_s[pl.ds(pl.multiple_of(b * 8, 8), 8), :].astype(BF16)
        return acc + jnp.dot(lhs, wd_s[rows, :], preferred_element_type=F32)
    y = lax.fori_loop(0, FB, down, jnp.zeros((8, D), F32))

    x8 = jnp.concatenate([xb_s[kb] for kb in range(KB)], axis=1)
    gate = sc_s[0][:, :1]
    rsel = sc_s[1][:, :1]
    out = gate * a + (1.0 - gate) * (x8 + y * rsel)
    o_ref[...] = out[0:B].astype(o_ref.dtype)


@jax.jit
def pallas_gated_mix__mha_block_cached__moe_arch_mod__decode_kernel(
    A_x: jax.Array,
    A_k_cache: jax.Array,
    A_v_cache: jax.Array,
    A_wq: jax.Array,
    A_wo: jax.Array,
    B_x: jax.Array,
    B_w_r: jax.Array,
    B_w_gate: jax.Array,
    B_w_up: jax.Array,
    B_w_down: jax.Array,
    gate_w: jax.Array,
):
    del B_x
    out = pl.pallas_call(
        _kernel,
        out_shape=jax.ShapeDtypeStruct((B, D), BF16),
        in_specs=[pl.BlockSpec(memory_space=pl.ANY)] * 10,
        out_specs=pl.BlockSpec(memory_space=pltpu.VMEM),
        scratch_shapes=[
            pltpu.VMEM((2 * NB, HG, R, DH), BF16),
            pltpu.VMEM((8, 128, H * DH), BF16),
            pltpu.VMEM((8, 512, D), BF16),
            pltpu.VMEM((2, 8, 128, F), BF16),
            pltpu.VMEM((F, D), BF16),
            pltpu.VMEM((B, D), BF16),
            pltpu.VMEM((D,), BF16),
            pltpu.VMEM((D,), BF16),
            pltpu.VMEM((KB, 8, 128), F32),
            pltpu.VMEM((H * 8, 128), F32),
            pltpu.VMEM((2 * B * H, 128), F32),
            pltpu.VMEM((FB * 8, 128), F32),
            pltpu.VMEM((FB * 8, 128), F32),
            pltpu.VMEM((2, 8, 128), F32),
            pltpu.VMEM((8, D), F32),
            pltpu.SemaphoreType.DMA((2 * NB,)),
            pltpu.SemaphoreType.DMA((7,)),
            pltpu.SemaphoreType.DMA((FB,)),
        ],
        compiler_params=pltpu.CompilerParams(vmem_limit_bytes=64 * 1024 * 1024),
    )(A_x.reshape(B, D), A_k_cache.reshape(G, HG, S, DH), A_v_cache.reshape(G, HG, S, DH),
      A_wq.reshape(8, 128, H * DH), A_wo.reshape(8, 512, D), B_w_r,
      B_w_gate.reshape(8, 128, F), B_w_up.reshape(8, 128, F), B_w_down, gate_w)
    return out.reshape(B, 1, D)
```

```python
import functools

import jax
import jax.numpy as jnp
from jax import lax
import jax.experimental.pallas as pl
import jax.experimental.pallas.tpu as pltpu

F32, BF16 = jnp.float32, jnp.bfloat16

B, D, H, S, DH, F = 4, 1024, 32, 8192, 128, 3584
HG = 8
G = B * H // HG
SCALE = DH ** -0.5
R = 128
SEG = 16
NS = S // R
T = G * NS
L = 14
NB = L + 1
KB = D // 128
FB = F // 128
WD_LAG = 5
WO_T0 = T - L - (H - HG)


def _kernel(x_hbm, k_hbm, v_hbm, wq_hbm, wo_hbm, wr_hbm, wg_hbm, wu_hbm, wd_hbm, gw_hbm, o_ref,
            kv, wq_s, wo_s, wgu_s, wd_s, x_s, wr_s, gw_s, xb_s, q_s, o_s, g_s, u_s, sc_s, a_s, y_s,
            sem_kv, sem_w, sem_wd):
    def kv_copy(t, j, which):
        base = pl.multiple_of((t % NS) * R, R)
        sl = which * NB + t % NB
        src = (k_hbm, v_hbm)[which]
        pltpu.make_async_copy(src.at[t // NS, :, pl.ds(base + j * SEG, SEG)],
                              kv.at[sl, :, pl.ds(j * SEG, SEG)], sem_kv.at[sl]).start(priority=which)

    def kv_dmas(t):
        return [functools.partial(kv_copy, t, j, w) for j in range(R // SEG) for w in (0, 1)]

    def wd_copy(blk, j, which):
        b = blk + which * (FB // 2)
        r = pl.multiple_of(b * 128 + j * 16, 16)
        pltpu.make_async_copy(wd_hbm.at[pl.ds(r, 16)], wd_s.at[pl.ds(r, 16)], sem_wd.at[b]).start(priority=which)

    def wd_dmas(blk):
        return [functools.partial(wd_copy, blk, j, w) for j in range(8) for w in (0, 1)]

    def wait_all(ref, sem):
        pltpu.make_async_copy(ref, ref, sem).wait()

    small = [pltpu.make_async_copy(x_hbm, x_s, sem_w.at[4]),
             pltpu.make_async_copy(wr_hbm, wr_s, sem_w.at[5]),
             pltpu.make_async_copy(gw_hbm, gw_s, sem_w.at[6])]
    for c in small:
        c.start()

    def p1(r8, c):
        r = pl.multiple_of(r8 * 8, 8)
        for cb in range(F // 256):
            for w, src in enumerate((wg_hbm, wu_hbm)):
                pltpu.make_async_copy(src.at[:, pl.ds(r, 8), pl.ds(cb * 256, 256)],
                                      wgu_s.at[w, :, pl.ds(r, 8), pl.ds(cb * 256, 256)],
                                      sem_w.at[w]).start(priority=w)
        return c
    lax.fori_loop(0, 16, p1, 0)

    for c in small:
        c.wait()
    x4 = x_s[...].astype(F32)
    x8 = jnp.concatenate([x4, jnp.zeros_like(x4)], axis=0)
    for kb in range(KB):
        xb_s[kb] = x8[:, kb * 128:(kb + 1) * 128]
    gate = jax.nn.sigmoid(jnp.sum(x8 * gw_s[...].astype(F32).reshape(1, D), axis=-1, keepdims=True))
    rsel = jax.nn.sigmoid(jnp.sum(x8 * wr_s[...].astype(F32).reshape(1, D), axis=-1, keepdims=True))
    sc_s[0] = jnp.broadcast_to(gate, (8, 128))
    sc_s[1] = jnp.broadcast_to(rsel, (8, 128))
    q_s[...] = jnp.zeros_like(q_s)
    g_s[...] = jnp.zeros_like(g_s)
    u_s[...] = jnp.zeros_like(u_s)
    o_s[...] = jnp.zeros_like(o_s)
    a_s[...] = jnp.zeros_like(a_s)
    y_s[...] = jnp.zeros_like(y_s)

    def p2_issue(r8):
        r = pl.multiple_of(r8 * 8, 8)
        for cb in range(16):
            pltpu.make_async_copy(wq_hbm.at[:, pl.ds(r, 8), pl.ds(cb * 256, 256)],
                                  wq_s.at[:, pl.ds(r, 8), pl.ds(cb * 256, 256)], sem_w.at[2]).start(priority=0)
            r0 = pl.multiple_of(r8 * 32 + (cb // 4) * 8, 8)
            c0 = (cb % 4) * 256
            pltpu.make_async_copy(wo_hbm.at[:, pl.ds(r0, 8), pl.ds(c0, 256)],
                                  wo_s.at[:, pl.ds(r0, 8), pl.ds(c0, 256)], sem_w.at[3]).start(priority=1)

    def acc_cols(dst, part):
        for j in range(part.shape[1] // 128):
            dst[j * 8:(j + 1) * 8, :] += part[:, j * 128:(j + 1) * 128]

    def p2a(r8, c):
        p2_issue(r8)
        return c
    lax.fori_loop(0, 8, p2a, 0)
    wait_all(wgu_s.at[0], sem_w.at[0])
    wait_all(wgu_s.at[1], sem_w.at[1])

    def p2b(r8, c):
        p2_issue(r8)
        kb = r8 - 8
        xk = xb_s[kb].astype(BF16)
        acc_cols(g_s, jnp.dot(xk, wgu_s[0, kb], preferred_element_type=F32))
        acc_cols(u_s, jnp.dot(xk, wgu_s[1, kb], preferred_element_type=F32))
        return c
    lax.fori_loop(8, 16, p2b, 0)

    def p3a(t, c):
        for d in kv_dmas(t):
            d()
        return c
    lax.fori_loop(0, L - KB, p3a, 0)
    gg = g_s[...]
    g_s[...] = gg * jax.nn.sigmoid(gg) * u_s[...]
    wait_all(wq_s, sem_w.at[2])

    def p3b(t, c):
        for d in kv_dmas(t):
            d()
        kb = t - (L - KB)
        acc_cols(q_s, jnp.dot(xb_s[kb].astype(BF16), wq_s[kb], preferred_element_type=F32))
        return c
    lax.fori_loop(L - KB, L, p3b, 0)

    neg = jnp.full((8, 128), -jnp.inf, F32)
    zero = jnp.zeros((8, 128), F32)
    row = lax.broadcasted_iota(jnp.int32, (8, R), 0)

    def finalize(g, l, acc):
        o_s[pl.ds(pl.multiple_of(g * 8, 8), 8), :] = acc / jnp.sum(l, axis=-1, keepdims=True)

    def wo_block(h):
        lhs = o_s[pl.ds(h, 8, stride=H), :].astype(BF16)
        w = wo_s[h // 4, pl.ds(pl.multiple_of((h % 4) * 128, 128), 128), :]
        return jnp.dot(lhs, w, preferred_element_type=F32)

    def wd_wait(b):
        wait_all(wd_s.at[pl.ds(pl.multiple_of(b * 128, 128), 128)], sem_wd.at[b])

    def wd_block(b):
        lhs = g_s[pl.ds(pl.multiple_of(b * 8, 8), 8), :].astype(BF16)
        return jnp.dot(lhs, wd_s[pl.ds(pl.multiple_of(b * 128, 128), 128), :], preferred_element_type=F32)

    def step(t, carry, dmas, fin):
        m, l, acc = carry
        g = t // NS
        c = t % NS
        ks, vs = t % NB, NB + t % NB
        wait_all(kv.at[ks], sem_kv.at[ks])
        wait_all(kv.at[vs], sem_kv.at[vs])
        first = c == 0
        m = jnp.where(first, neg, m)
        l = jnp.where(first, zero, l)
        acc = jnp.where(first, zero, acc)
        q = q_s[pl.ds((g % 4) * 64 + g // 4, 8, stride=8), :].astype(BF16)
        s = None
        for j in range(HG):
            dmas[j]()
            sj = lax.dot_general(q, kv[ks, j], (((1,), (1,)), ((), ())), preferred_element_type=F32)
            s = sj if s is None else jnp.where(row == j, sj, s)
        s = s * SCALE
        m_new = jnp.maximum(m, jnp.max(s, axis=-1, keepdims=True))
        alpha = jnp.exp(m - m_new)
        p = jnp.exp(s - m_new)
        l = l * alpha + p
        pv = None
        for j in range(HG):
            dmas[HG + j]()
            pj = jnp.where(row == j, p, 0.0).astype(BF16)
            d = jnp.dot(pj, kv[vs, j], preferred_element_type=F32)
            pv = d if pv is None else pv + d
        acc = acc * alpha + pv
        if fin:
            @pl.when(c == NS - 1)
            def _():
                finalize(g, l, acc)

            @pl.when(t >= WO_T0)
            def _():
                a_s[...] += wo_block(t - WO_T0)
        return m_new, l, acc

    wait_all(wo_s, sem_w.at[3])
    cr = lax.fori_loop(0, T - L, lambda t, cr: step(t, cr, kv_dmas(t + L), True), (neg, zero, zero))

    def tail(it, cr, with_wd):
        if with_wd:
            wd_wait(it - WD_LAG)
        cr = step(T - L + it, cr, wd_dmas(it), False)
        if with_wd:
            y_s[...] += wd_block(it - WD_LAG)
        return cr
    cr = lax.fori_loop(0, WD_LAG, lambda it, cr: tail(it, cr, False), cr)
    cr = lax.fori_loop(WD_LAG, L, lambda it, cr: tail(it, cr, True), cr)
    finalize(G - 1, cr[1], cr[2])
    a = a_s[...]
    for h in range(H - HG, H):
        a = a + wo_block(h)

    lo0, hi0 = L - 4, FB - 7
    landed = list(range(L - WD_LAG, lo0)) + list(range(L, hi0))
    for b in landed:
        wd_wait(b)
    y = y_s[...]
    for b in landed:
        y = y + wd_block(b)

    def down(b, acc):
        wd_wait(b)
        return acc + wd_block(b)
    y = lax.fori_loop(0, 8, lambda i, acc: down(lo0 + i // 2 + (i % 2) * (hi0 - lo0), acc), y)
    y = lax.fori_loop(FB - 3, FB, down, y)

    x8 = jnp.concatenate([xb_s[kb] for kb in range(KB)], axis=1)
    gate = sc_s[0][:, :1]
    rsel = sc_s[1][:, :1]
    out = gate * a + (1.0 - gate) * (x8 + y * rsel)
    o_ref[...] = out[0:B].astype(o_ref.dtype)


@jax.jit
def pallas_gated_mix__mha_block_cached__moe_arch_mod__decode_kernel(
    A_x: jax.Array,
    A_k_cache: jax.Array,
    A_v_cache: jax.Array,
    A_wq: jax.Array,
    A_wo: jax.Array,
    B_x: jax.Array,
    B_w_r: jax.Array,
    B_w_gate: jax.Array,
    B_w_up: jax.Array,
    B_w_down: jax.Array,
    gate_w: jax.Array,
):
    del B_x
    out = pl.pallas_call(
        _kernel,
        out_shape=jax.ShapeDtypeStruct((B, D), BF16),
        in_specs=[pl.BlockSpec(memory_space=pl.ANY)] * 10,
        out_specs=pl.BlockSpec(memory_space=pltpu.VMEM),
        scratch_shapes=[
            pltpu.VMEM((2 * NB, HG, R, DH), BF16),
            pltpu.VMEM((8, 128, H * DH), BF16),
            pltpu.VMEM((8, 512, D), BF16),
            pltpu.VMEM((2, 8, 128, F), BF16),
            pltpu.VMEM((F, D), BF16),
            pltpu.VMEM((B, D), BF16),
            pltpu.VMEM((D,), BF16),
            pltpu.VMEM((D,), BF16),
            pltpu.VMEM((KB, 8, 128), F32),
            pltpu.VMEM((H * 8, 128), F32),
            pltpu.VMEM((2 * B * H, 128), F32),
            pltpu.VMEM((FB * 8, 128), F32),
            pltpu.VMEM((FB * 8, 128), F32),
            pltpu.VMEM((2, 8, 128), F32),
            pltpu.VMEM((8, D), F32),
            pltpu.VMEM((8, D), F32),
            pltpu.SemaphoreType.DMA((2 * NB,)),
            pltpu.SemaphoreType.DMA((7,)),
            pltpu.SemaphoreType.DMA((FB,)),
        ],
        compiler_params=pltpu.CompilerParams(vmem_limit_bytes=64 * 1024 * 1024,
                                             disable_semaphore_checks=True),
    )(A_x.reshape(B, D), A_k_cache.reshape(G, HG, S, DH), A_v_cache.reshape(G, HG, S, DH),
      A_wq.reshape(8, 128, H * DH), A_wo.reshape(8, 512, D), B_w_r,
      B_w_gate.reshape(8, 128, F), B_w_up.reshape(8, 128, F), B_w_down, gate_w)
    return out.reshape(B, 1, D)
```

```python
import functools

import jax
import jax.numpy as jnp
from jax import lax
import jax.experimental.pallas as pl
import jax.experimental.pallas.tpu as pltpu

F32, BF16 = jnp.float32, jnp.bfloat16

B, D, H, S, DH, F = 4, 1024, 32, 8192, 128, 3584
HG = 8
G = B * H // HG
SCALE = DH ** -0.5
R = 128
SEG = 16
NS = S // R
T = G * NS
SKEW = 3
LK = 6
LV = LK + SKEW
NBK, NBV = LK + 1, LV + 1
KB = D // 128
FB = F // 128
WD_EARLY = 16
WD_END = WD_EARLY + SKEW
WO_T0 = T - LV - (H - HG)


def _kernel(x_hbm, k_hbm, v_hbm, wq_hbm, wo_hbm, wr_hbm, wg_hbm, wu_hbm, wd_hbm, gw_hbm, o_ref,
            kv, wq_s, wo_s, wgu_s, wd_s, x_s, wr_s, gw_s, xb_s, q_s, o_s, gu_s, h_s, sc_s, a_s, y_s,
            sem_kv, sem_w, sem_wd):
    def slot(t, which):
        return t % NBK if which == 0 else NBK + t % NBV

    def kv_copy(t, which, j):
        base = pl.multiple_of((t % NS) * R, R)
        sl = slot(t, which)
        src = (k_hbm, v_hbm)[which]
        pltpu.make_async_copy(src.at[t // NS, :, pl.ds(base + j * SEG, SEG)],
                              kv.at[sl, :, pl.ds(j * SEG, SEG)], sem_kv.at[sl]).start(priority=which)

    def wd_copy(b, prio, j):
        r = pl.multiple_of((b % 4) * 128 + j * 16, 16)
        pltpu.make_async_copy(wd_hbm.at[b // 4, pl.ds(r, 16)], wd_s.at[b // 4, pl.ds(r, 16)],
                              sem_wd.at[b - WD_EARLY]).start(priority=prio)

    k_of = lambda t: functools.partial(kv_copy, t, 0)
    v_of = lambda t: functools.partial(kv_copy, t, 1)
    wd_of = lambda b, prio: functools.partial(wd_copy, b, prio)

    def pairs(hi, lo):
        return [functools.partial(f, j) for j in range(8) for f in (hi, lo)]

    def issue(dmas):
        for d in dmas:
            d()

    def loop(lo, hi, body):
        def wrapped(i, c):
            body(i)
            return c
        lax.fori_loop(lo, hi, wrapped, 0)

    def wait_all(ref, sem):
        pltpu.make_async_copy(ref, ref, sem).wait()

    def wd_rows(b):
        return wd_s.at[b // 4, pl.ds(pl.multiple_of((b % 4) * 128, 128), 128)]

    def wd_wait(b):
        wait_all(wd_rows(b), sem_wd.at[b - WD_EARLY])

    small = [pltpu.make_async_copy(x_hbm, x_s, sem_w.at[4]),
             pltpu.make_async_copy(wr_hbm, wr_s, sem_w.at[5]),
             pltpu.make_async_copy(gw_hbm, gw_s, sem_w.at[6])]
    for c in small:
        c.start()

    def issue_gate_up(r8):
        r = pl.multiple_of(r8 * 8, 8)
        for cb in range(F // 256):
            for w, src in enumerate((wg_hbm, wu_hbm)):
                pltpu.make_async_copy(src.at[:, pl.ds(r, 8), pl.ds(cb * 256, 256)],
                                      wgu_s.at[w, :, pl.ds(r, 8), pl.ds(cb * 256, 256)],
                                      sem_w.at[w]).start(priority=w)
    loop(0, 16, issue_gate_up)

    def issue_down(i):
        for rr in range(4):
            for cc in range(2):
                for w in range(2):
                    r = pl.multiple_of(w * 256 + (i * 4 + rr) * 8, 8)
                    pltpu.make_async_copy(wd_hbm.at[0:4, pl.ds(r, 8), pl.ds(cc * 512, 512)],
                                          wd_s.at[0:4, pl.ds(r, 8), pl.ds(cc * 512, 512)],
                                          sem_w.at[7]).start(priority=w)
    loop(0, 8, issue_down)

    for c in small:
        c.wait()
    x4 = x_s[...].astype(F32)
    x8 = jnp.concatenate([x4, jnp.zeros_like(x4)], axis=0)
    for kb in range(KB):
        xb_s[kb] = x8[:, kb * 128:(kb + 1) * 128]
    gate = jax.nn.sigmoid(jnp.sum(x8 * gw_s[...].astype(F32).reshape(1, D), axis=-1, keepdims=True))
    rsel = jax.nn.sigmoid(jnp.sum(x8 * wr_s[...].astype(F32).reshape(1, D), axis=-1, keepdims=True))
    sc_s[0] = jnp.broadcast_to(gate, (8, 128))
    sc_s[1] = jnp.broadcast_to(rsel, (8, 128))
    q_s[...] = jnp.zeros_like(q_s)
    gu_s[...] = jnp.zeros_like(gu_s)
    o_s[...] = jnp.zeros_like(o_s)
    a_s[...] = jnp.zeros_like(a_s)
    y_s[...] = jnp.zeros_like(y_s)

    def issue_q_o(r8):
        r = pl.multiple_of(r8 * 8, 8)
        for cb in range(16):
            pltpu.make_async_copy(wq_hbm.at[:, pl.ds(r, 8), pl.ds(cb * 256, 256)],
                                  wq_s.at[:, pl.ds(r, 8), pl.ds(cb * 256, 256)], sem_w.at[2]).start(priority=0)
            r0 = pl.multiple_of(r8 * 32 + (cb // 4) * 8, 8)
            c0 = (cb % 4) * 256
            pltpu.make_async_copy(wo_hbm.at[:, pl.ds(r0, 8), pl.ds(c0, 256)],
                                  wo_s.at[:, pl.ds(r0, 8), pl.ds(c0, 256)], sem_w.at[3]).start(priority=1)

    def acc_cols(dst, part):
        for j in range(part.shape[1] // 128):
            dst[j * 8:(j + 1) * 8, :] += part[:, j * 128:(j + 1) * 128]

    loop(0, 8, issue_q_o)
    wait_all(wgu_s.at[0], sem_w.at[0])
    wait_all(wgu_s.at[1], sem_w.at[1])

    def gate_up(r8):
        issue_q_o(r8)
        kb = r8 - 8
        xk = xb_s[kb].astype(BF16)
        acc_cols(gu_s.at[0], jnp.dot(xk, wgu_s[0, kb], preferred_element_type=F32))
        acc_cols(gu_s.at[1], jnp.dot(xk, wgu_s[1, kb], preferred_element_type=F32))
    loop(8, 16, gate_up)

    loop(0, SKEW, lambda t: issue(pairs(wd_of(WD_EARLY + t, 0), v_of(t))))
    gg = gu_s[0]
    h_s[...] = gg * jax.nn.sigmoid(gg) * gu_s[1]
    loop(0, LK - KB // 2, lambda t: issue(pairs(k_of(t), v_of(t + SKEW))))
    wait_all(wq_s, sem_w.at[2])

    def q_proj(t):
        issue(pairs(k_of(t), v_of(t + SKEW)))
        kb = (t - (LK - KB // 2)) * 2
        acc_cols(q_s, jnp.dot(xb_s[kb].astype(BF16), wq_s[kb], preferred_element_type=F32)
                 + jnp.dot(xb_s[kb + 1].astype(BF16), wq_s[kb + 1], preferred_element_type=F32))
    loop(LK - KB // 2, LK, q_proj)

    neg = jnp.full((8, 128), -jnp.inf, F32)
    zero = jnp.zeros((8, 128), F32)
    row = lax.broadcasted_iota(jnp.int32, (8, R), 0)

    def wo_block(h):
        lhs = o_s[pl.ds(h, 8, stride=H), :].astype(BF16)
        w = wo_s[h // 4, pl.ds(pl.multiple_of((h % 4) * 128, 128), 128), :]
        return jnp.dot(lhs, w, preferred_element_type=F32)

    def wd_block(b):
        lhs = h_s[pl.ds(pl.multiple_of(b * 8, 8), 8), :].astype(BF16)
        return jnp.dot(lhs, wd_rows(b)[...], preferred_element_type=F32)

    def finalize(g, l, acc):
        o_s[pl.ds(pl.multiple_of(g * 8, 8), 8), :] = acc / jnp.sum(l, axis=-1, keepdims=True)

    def step(t, carry, dmas):
        m, l, acc = carry
        g = t // NS
        ks, vs = slot(t, 0), slot(t, 1)
        wait_all(kv.at[ks], sem_kv.at[ks])
        wait_all(kv.at[vs], sem_kv.at[vs])
        first = t % NS == 0
        m = jnp.where(first, neg, m)
        l = jnp.where(first, zero, l)
        acc = jnp.where(first, zero, acc)
        q = q_s[pl.ds((g % 4) * 64 + g // 4, 8, stride=8), :].astype(BF16)
        s = None
        for j in range(HG):
            issue(dmas[j:j + 1])
            sj = lax.dot_general(q, kv[ks, j], (((1,), (1,)), ((), ())), preferred_element_type=F32)
            s = sj if s is None else jnp.where(row == j, sj, s)
        s = s * SCALE
        m_new = jnp.maximum(m, jnp.max(s, axis=-1, keepdims=True))
        alpha = jnp.exp(m - m_new)
        p = jnp.exp(s - m_new)
        l = l * alpha + p
        pv = None
        for j in range(HG):
            issue(dmas[HG + j:HG + j + 1])
            pj = jnp.where(row == j, p, 0.0).astype(BF16)
            d = jnp.dot(pj, kv[vs, j], preferred_element_type=F32)
            pv = d if pv is None else pv + d
        return m_new, l, acc * alpha + pv

    def main_step(t, cr):
        cr = step(t, cr, pairs(k_of(t + LK), v_of(t + LV)))

        @pl.when(t % NS == NS - 1)
        def _():
            finalize(t // NS, cr[1], cr[2])

        @pl.when(t < WD_END)
        def _():
            y_s[...] += wd_block(t)

        @pl.when(t >= WO_T0)
        def _():
            a_s[...] += wo_block(t - WO_T0)
        return cr

    wait_all(wo_s, sem_w.at[3])
    wait_all(wd_s.at[0:4], sem_w.at[7])
    for b in range(WD_EARLY, WD_END):
        wd_wait(b)
    cr = lax.fori_loop(0, T - LV, main_step, (neg, zero, zero))

    def tail_step(it, cr):
        t = T - LV + it

        @pl.when(it < SKEW)
        def _():
            issue(pairs(k_of(t + LK), wd_of(WD_END + 1 + 2 * it, 1)))

        @pl.when(jnp.logical_and(it >= SKEW, it < 2 * SKEW))
        def _():
            issue(pairs(wd_of(WD_END + 2 * (it - SKEW), 0), wd_of(WD_END + SKEW + it, 1)))
        return step(t, cr, [])
    cr = lax.fori_loop(0, LV, tail_step, cr)
    finalize(G - 1, cr[1], cr[2])
    a = a_s[...]
    for h in range(H - HG, H):
        a = a + wo_block(h)

    def down(b, acc):
        wd_wait(b)
        return acc + wd_block(b)
    y = lax.fori_loop(WD_END, FB, down, y_s[...])

    x8 = jnp.concatenate([xb_s[kb] for kb in range(KB)], axis=1)
    gate = sc_s[0][:, :1]
    rsel = sc_s[1][:, :1]
    out = gate * a + (1.0 - gate) * (x8 + y * rsel)
    o_ref[...] = out[0:B].astype(o_ref.dtype)


@jax.jit
def pallas_gated_mix__mha_block_cached__moe_arch_mod__decode_kernel(
    A_x: jax.Array,
    A_k_cache: jax.Array,
    A_v_cache: jax.Array,
    A_wq: jax.Array,
    A_wo: jax.Array,
    B_x: jax.Array,
    B_w_r: jax.Array,
    B_w_gate: jax.Array,
    B_w_up: jax.Array,
    B_w_down: jax.Array,
    gate_w: jax.Array,
):
    del B_x
    out = pl.pallas_call(
        _kernel,
        out_shape=jax.ShapeDtypeStruct((B, D), BF16),
        in_specs=[pl.BlockSpec(memory_space=pl.ANY)] * 10,
        out_specs=pl.BlockSpec(memory_space=pltpu.VMEM),
        scratch_shapes=[
            pltpu.VMEM((NBK + NBV, HG, R, DH), BF16),
            pltpu.VMEM((8, 128, H * DH), BF16),
            pltpu.VMEM((8, 512, D), BF16),
            pltpu.VMEM((2, 8, 128, F), BF16),
            pltpu.VMEM((7, 512, D), BF16),
            pltpu.VMEM((B, D), BF16),
            pltpu.VMEM((D,), BF16),
            pltpu.VMEM((D,), BF16),
            pltpu.VMEM((KB, 8, 128), F32),
            pltpu.VMEM((H * 8 + 8, 128), F32),
            pltpu.VMEM((2 * B * H + H, 128), F32),
            pltpu.VMEM((2, FB * 8, 128), F32),
            pltpu.VMEM((FB * 8, 128), F32),
            pltpu.VMEM((2, 8, 128), F32),
            pltpu.VMEM((8, D), F32),
            pltpu.VMEM((8, D), F32),
            pltpu.SemaphoreType.DMA((NBK + NBV,)),
            pltpu.SemaphoreType.DMA((8,)),
            pltpu.SemaphoreType.DMA((FB - WD_EARLY,)),
        ],
        compiler_params=pltpu.CompilerParams(vmem_limit_bytes=64 * 1024 * 1024,
                                             disable_semaphore_checks=True),
    )(A_x.reshape(B, D), A_k_cache.reshape(G, HG, S, DH), A_v_cache.reshape(G, HG, S, DH),
      A_wq.reshape(8, 128, H * DH), A_wo.reshape(8, 512, D), B_w_r,
      B_w_gate.reshape(8, 128, F), B_w_up.reshape(8, 128, F), B_w_down.reshape(7, 512, D), gate_w)
    return out.reshape(B, 1, D)
```

```python
import dataclasses
import functools

import jax
import jax.numpy as jnp
from jax import lax
import jax.experimental.pallas as pl
import jax.experimental.pallas.tpu as pltpu

F32, BF16 = jnp.float32, jnp.bfloat16

B, D, H, S, DH, F = 4, 1024, 32, 8192, 128, 3584
HG = 8
G = B * H // HG
SCALE = DH ** -0.5
R = 128
SEG = 16
NS = S // R
T = G * NS
SKEW = 3
LK = 6
LV = LK + SKEW
NBK, NBV = LK + 1, LV + 1
KB = D // 128
FB = F // 128
WD_EARLY = 16
WD_END = WD_EARLY + SKEW
WO_T0 = T - LV - (H - HG)


_PARAMS = dict(vmem_limit_bytes=64 * 1024 * 1024)
if any(f.name == "disable_semaphore_checks" for f in dataclasses.fields(pltpu.CompilerParams)):
    _PARAMS["disable_semaphore_checks"] = True


def _kernel(x_hbm, k_hbm, v_hbm, wq_hbm, wo_hbm, wr_hbm, wg_hbm, wu_hbm, wd_hbm, gw_hbm, o_ref,
            kv, wq_s, wo_s, wgu_s, wd_s, x_s, wr_s, gw_s, xb_s, q_s, o_s, gu_s, h_s, sc_s, a_s, y_s,
            sem_kv, sem_w, sem_wd):
    def slot(t, which):
        return t % NBK if which == 0 else NBK + t % NBV

    def kv_copy(t, which, j):
        base = pl.multiple_of((t % NS) * R, R)
        sl = slot(t, which)
        src = (k_hbm, v_hbm)[which]
        pltpu.make_async_copy(src.at[t // NS, :, pl.ds(base + j * SEG, SEG)],
                              kv.at[sl, :, pl.ds(j * SEG, SEG)], sem_kv.at[sl]).start(priority=which)

    def wd_copy(b, prio, j):
        r = pl.multiple_of((b % 4) * 128 + j * 16, 16)
        pltpu.make_async_copy(wd_hbm.at[b // 4, pl.ds(r, 16)], wd_s.at[b // 4, pl.ds(r, 16)],
                              sem_wd.at[b - WD_EARLY]).start(priority=prio)

    k_of = lambda t: functools.partial(kv_copy, t, 0)
    v_of = lambda t: functools.partial(kv_copy, t, 1)
    wd_of = lambda b, prio: functools.partial(wd_copy, b, prio)

    def pairs(hi, lo):
        return [functools.partial(f, j) for j in range(8) for f in (hi, lo)]

    def issue(dmas):
        for d in dmas:
            d()

    def loop(lo, hi, body):
        def wrapped(i, c):
            body(i)
            return c
        lax.fori_loop(lo, hi, wrapped, 0)

    def wait_all(ref, sem):
        pltpu.make_async_copy(ref, ref, sem).wait()

    def wd_rows(b):
        return wd_s.at[b // 4, pl.ds(pl.multiple_of((b % 4) * 128, 128), 128)]

    def wd_wait(b):
        wait_all(wd_rows(b), sem_wd.at[b - WD_EARLY])

    small = [pltpu.make_async_copy(x_hbm, x_s, sem_w.at[4]),
             pltpu.make_async_copy(wr_hbm, wr_s, sem_w.at[5]),
             pltpu.make_async_copy(gw_hbm, gw_s, sem_w.at[6])]
    for c in small:
        c.start()

    def issue_gate_up(r8):
        r = pl.multiple_of(r8 * 8, 8)
        for cb in range(F // 256):
            for w, src in enumerate((wg_hbm, wu_hbm)):
                pltpu.make_async_copy(src.at[:, pl.ds(r, 8), pl.ds(cb * 256, 256)],
                                      wgu_s.at[w, :, pl.ds(r, 8), pl.ds(cb * 256, 256)],
                                      sem_w.at[w]).start(priority=w)
    loop(0, 16, issue_gate_up)

    def issue_down(i):
        for rr in range(4):
            for cc in range(2):
                for w in range(2):
                    r = pl.multiple_of(w * 256 + (i * 4 + rr) * 8, 8)
                    pltpu.make_async_copy(wd_hbm.at[0:4, pl.ds(r, 8), pl.ds(cc * 512, 512)],
                                          wd_s.at[0:4, pl.ds(r, 8), pl.ds(cc * 512, 512)],
                                          sem_w.at[7]).start(priority=w)
    loop(0, 8, issue_down)

    for c in small:
        c.wait()
    x4 = x_s[...].astype(F32)
    x8 = jnp.concatenate([x4, jnp.zeros_like(x4)], axis=0)
    for kb in range(KB):
        xb_s[kb] = x8[:, kb * 128:(kb + 1) * 128]
    gate = jax.nn.sigmoid(jnp.sum(x8 * gw_s[...].astype(F32).reshape(1, D), axis=-1, keepdims=True))
    rsel = jax.nn.sigmoid(jnp.sum(x8 * wr_s[...].astype(F32).reshape(1, D), axis=-1, keepdims=True))
    sc_s[0] = jnp.broadcast_to(gate, (8, 128))
    sc_s[1] = jnp.broadcast_to(rsel, (8, 128))
    q_s[...] = jnp.zeros_like(q_s)
    gu_s[...] = jnp.zeros_like(gu_s)
    o_s[...] = jnp.zeros_like(o_s)
    a_s[...] = jnp.zeros_like(a_s)
    y_s[...] = jnp.zeros_like(y_s)

    def issue_q_o(r8):
        r = pl.multiple_of(r8 * 8, 8)
        for cb in range(16):
            pltpu.make_async_copy(wq_hbm.at[:, pl.ds(r, 8), pl.ds(cb * 256, 256)],
                                  wq_s.at[:, pl.ds(r, 8), pl.ds(cb * 256, 256)], sem_w.at[2]).start(priority=0)
            r0 = pl.multiple_of(r8 * 32 + (cb // 4) * 8, 8)
            c0 = (cb % 4) * 256
            pltpu.make_async_copy(wo_hbm.at[:, pl.ds(r0, 8), pl.ds(c0, 256)],
                                  wo_s.at[:, pl.ds(r0, 8), pl.ds(c0, 256)], sem_w.at[3]).start(priority=1)

    def acc_cols(dst, part):
        for j in range(part.shape[1] // 128):
            dst[j * 8:(j + 1) * 8, :] += part[:, j * 128:(j + 1) * 128]

    loop(0, 8, issue_q_o)
    wait_all(wgu_s.at[0], sem_w.at[0])
    wait_all(wgu_s.at[1], sem_w.at[1])

    def gate_up(r8):
        issue_q_o(r8)
        kb = r8 - 8
        xk = xb_s[kb].astype(BF16)
        acc_cols(gu_s.at[0], jnp.dot(xk, wgu_s[0, kb], preferred_element_type=F32))
        acc_cols(gu_s.at[1], jnp.dot(xk, wgu_s[1, kb], preferred_element_type=F32))
    loop(8, 16, gate_up)

    loop(0, SKEW, lambda t: issue(pairs(wd_of(WD_EARLY + t, 0), v_of(t))))
    gg = gu_s[0]
    h_s[...] = gg * jax.nn.sigmoid(gg) * gu_s[1]
    loop(0, LK - KB // 2, lambda t: issue(pairs(k_of(t), v_of(t + SKEW))))
    wait_all(wq_s, sem_w.at[2])

    def q_proj(t):
        issue(pairs(k_of(t), v_of(t + SKEW)))
        kb = (t - (LK - KB // 2)) * 2
        acc_cols(q_s, jnp.dot(xb_s[kb].astype(BF16), wq_s[kb], preferred_element_type=F32)
                 + jnp.dot(xb_s[kb + 1].astype(BF16), wq_s[kb + 1], preferred_element_type=F32))
    loop(LK - KB // 2, LK, q_proj)

    neg = jnp.full((8, 128), -jnp.inf, F32)
    zero = jnp.zeros((8, 128), F32)
    row = lax.broadcasted_iota(jnp.int32, (8, R), 0)

    def wo_block(h):
        lhs = o_s[pl.ds(h, 8, stride=H), :].astype(BF16)
        w = wo_s[h // 4, pl.ds(pl.multiple_of((h % 4) * 128, 128), 128), :]
        return jnp.dot(lhs, w, preferred_element_type=F32)

    def wd_block(b):
        lhs = h_s[pl.ds(pl.multiple_of(b * 8, 8), 8), :].astype(BF16)
        return jnp.dot(lhs, wd_rows(b)[...], preferred_element_type=F32)

    def finalize(g, l, acc):
        o_s[pl.ds(pl.multiple_of(g * 8, 8), 8), :] = acc / jnp.sum(l, axis=-1, keepdims=True)

    def step(t, carry, dmas):
        m, l, acc = carry
        g = t // NS
        ks, vs = slot(t, 0), slot(t, 1)
        wait_all(kv.at[ks], sem_kv.at[ks])
        wait_all(kv.at[vs], sem_kv.at[vs])
        first = t % NS == 0
        m = jnp.where(first, neg, m)
        l = jnp.where(first, zero, l)
        acc = jnp.where(first, zero, acc)
        q = q_s[pl.ds((g % 4) * 64 + g // 4, 8, stride=8), :].astype(BF16)
        s = None
        for j in range(HG):
            issue(dmas[j:j + 1])
            sj = lax.dot_general(q, kv[ks, j], (((1,), (1,)), ((), ())), preferred_element_type=F32)
            s = sj if s is None else jnp.where(row == j, sj, s)
        s = s * SCALE
        m_new = jnp.maximum(m, jnp.max(s, axis=-1, keepdims=True))
        alpha = jnp.exp(m - m_new)
        p = jnp.exp(s - m_new)
        l = l * alpha + p
        pv = None
        for j in range(HG):
            issue(dmas[HG + j:HG + j + 1])
            pj = jnp.where(row == j, p, 0.0).astype(BF16)
            d = jnp.dot(pj, kv[vs, j], preferred_element_type=F32)
            pv = d if pv is None else pv + d
        return m_new, l, acc * alpha + pv

    def main_step(t, cr):
        cr = step(t, cr, pairs(k_of(t + LK), v_of(t + LV)))

        @pl.when(t % NS == NS - 1)
        def _():
            finalize(t // NS, cr[1], cr[2])

        @pl.when(t < WD_END)
        def _():
            y_s[...] += wd_block(t)

        @pl.when(t >= WO_T0)
        def _():
            a_s[...] += wo_block(t - WO_T0)
        return cr

    wait_all(wo_s, sem_w.at[3])
    wait_all(wd_s.at[0:4], sem_w.at[7])
    for b in range(WD_EARLY, WD_END):
        wd_wait(b)
    cr = lax.fori_loop(0, T - LV, main_step, (neg, zero, zero))

    def tail_step(it, cr):
        t = T - LV + it

        @pl.when(it < SKEW)
        def _():
            issue(pairs(k_of(t + LK), wd_of(WD_END + 1 + 2 * it, 1)))

        @pl.when(jnp.logical_and(it >= SKEW, it < 2 * SKEW))
        def _():
            issue(pairs(wd_of(WD_END + 2 * (it - SKEW), 0), wd_of(WD_END + SKEW + it, 1)))
        return step(t, cr, [])
    cr = lax.fori_loop(0, LV, tail_step, cr)
    finalize(G - 1, cr[1], cr[2])
    a = a_s[...]
    for h in range(H - HG, H):
        a = a + wo_block(h)

    def down(b, acc):
        wd_wait(b)
        return acc + wd_block(b)
    y = lax.fori_loop(WD_END, FB, down, y_s[...])

    x8 = jnp.concatenate([xb_s[kb] for kb in range(KB)], axis=1)
    gate = sc_s[0][:, :1]
    rsel = sc_s[1][:, :1]
    out = gate * a + (1.0 - gate) * (x8 + y * rsel)
    o_ref[...] = out[0:B].astype(o_ref.dtype)


@jax.jit
def pallas_gated_mix__mha_block_cached__moe_arch_mod__decode_kernel(
    A_x: jax.Array,
    A_k_cache: jax.Array,
    A_v_cache: jax.Array,
    A_wq: jax.Array,
    A_wo: jax.Array,
    B_x: jax.Array,
    B_w_r: jax.Array,
    B_w_gate: jax.Array,
    B_w_up: jax.Array,
    B_w_down: jax.Array,
    gate_w: jax.Array,
):
    del B_x
    out = pl.pallas_call(
        _kernel,
        out_shape=jax.ShapeDtypeStruct((B, D), BF16),
        in_specs=[pl.BlockSpec(memory_space=pl.ANY)] * 10,
        out_specs=pl.BlockSpec(memory_space=pltpu.VMEM),
        scratch_shapes=[
            pltpu.VMEM((NBK + NBV, HG, R, DH), BF16),
            pltpu.VMEM((8, 128, H * DH), BF16),
            pltpu.VMEM((8, 512, D), BF16),
            pltpu.VMEM((2, 8, 128, F), BF16),
            pltpu.VMEM((7, 512, D), BF16),
            pltpu.VMEM((B, D), BF16),
            pltpu.VMEM((D,), BF16),
            pltpu.VMEM((D,), BF16),
            pltpu.VMEM((KB, 8, 128), F32),
            pltpu.VMEM((H * 8 + 8, 128), F32),
            pltpu.VMEM((2 * B * H + H, 128), F32),
            pltpu.VMEM((2, FB * 8, 128), F32),
            pltpu.VMEM((FB * 8, 128), F32),
            pltpu.VMEM((2, 8, 128), F32),
            pltpu.VMEM((8, D), F32),
            pltpu.VMEM((8, D), F32),
            pltpu.SemaphoreType.DMA((NBK + NBV,)),
            pltpu.SemaphoreType.DMA((8,)),
            pltpu.SemaphoreType.DMA((FB - WD_EARLY,)),
        ],
        compiler_params=pltpu.CompilerParams(**_PARAMS),
    )(A_x.reshape(B, D), A_k_cache.reshape(G, HG, S, DH), A_v_cache.reshape(G, HG, S, DH),
      A_wq.reshape(8, 128, H * DH), A_wo.reshape(8, 512, D), B_w_r,
      B_w_gate.reshape(8, 128, F), B_w_up.reshape(8, 128, F), B_w_down.reshape(7, 512, D), gate_w)
    return out.reshape(B, 1, D)
```

```python
import dataclasses
from functools import partial

import jax
import jax.numpy as jnp
from jax import lax
import jax.experimental.pallas as pl
import jax.experimental.pallas.tpu as pltpu

F32, BF16 = jnp.float32, jnp.bfloat16

B, D, H, S, DH, F = 4, 1024, 32, 8192, 128, 3584
HG = 8
G = B * H // HG
SCALE = DH ** -0.5
R = 128
SEG = 16
NS = S // R
T = G * NS
SKEW = 3
LK = 6
LV = LK + SKEW
NBK, NBV = LK + 1, LV + 1
KB = D // 128
FB = F // 128
BANDS = 5
WD_END = 4 * BANDS
WO_T0 = T - LV - (H - HG)

_PARAMS = dict(vmem_limit_bytes=64 * 1024 * 1024, disable_bounds_checks=True)
if any(f.name == "disable_semaphore_checks" for f in dataclasses.fields(pltpu.CompilerParams)):
    _PARAMS["disable_semaphore_checks"] = True


def _kernel(x_hbm, k_hbm, v_hbm, wq_hbm, wo_hbm, wr_hbm, wg_hbm, wu_hbm, wd_hbm, gw_hbm, o_ref,
            kv, wq_s, wo_s, wgu_s, wd_s, x_s, wr_s, gw_s, xb_s, q_s, o_s, gu_s, h_s, sc_s, a_s, y_s,
            sem_kv, sem_w, sem_wd):
    def band_copy(src, dst, r, c, cols, sem, prio):
        r = pl.multiple_of(r, 8)
        pltpu.make_async_copy(src.at[:, pl.ds(r, 8), pl.ds(c, cols)],
                              dst.at[:, pl.ds(r, 8), pl.ds(c, cols)], sem).start(priority=prio)

    def gate_up_copy(w, u, j):
        d = u * 8 + j
        band_copy((wg_hbm, wu_hbm)[w], wgu_s.at[w], (d // 14) * 8, pl.multiple_of((d % 14) * 256, 256), 256,
                  sem_w.at[w], w)

    def wq_copy(u, j):
        band_copy(wq_hbm, wq_s, (u // 2) * 8, pl.multiple_of(((u % 2) * 8 + j) * 256, 256), 256, sem_w.at[2], 0)

    def wo_copy(u, j):
        band_copy(wo_hbm, wo_s, (2 * u + j // 4) * 8, (j % 4) * 256, 256, sem_w.at[3], 1)

    def wd_band_copy(w, u, j):
        band_copy(wd_hbm.at[0:BANDS], wd_s.at[0:BANDS], w * 256 + (4 * u + j // 2) * 8, (j % 2) * 512, 512,
                  sem_w.at[7], w)

    def wd_copy(b, prio, j):
        r = pl.multiple_of((b % 4) * 128 + j * 16, 16)
        pltpu.make_async_copy(wd_hbm.at[b // 4, pl.ds(r, 16)], wd_s.at[b // 4, pl.ds(r, 16)],
                              sem_wd.at[b - WD_END]).start(priority=prio)

    def slot(t, which):
        return t % NBK if which == 0 else NBK + t % NBV

    def kv_copy(which, t, j):
        base = pl.multiple_of((t % NS) * R, R)
        sl = slot(t, which)
        pltpu.make_async_copy((k_hbm, v_hbm)[which].at[t // NS, :, pl.ds(base + j * SEG, SEG)],
                              kv.at[sl, :, pl.ds(j * SEG, SEG)], sem_kv.at[sl]).start(priority=which)

    def pairs(q0, q1):
        return [partial(f, j) for j in range(8) for f in (q0, q1)]

    def issue(dmas):
        for d in dmas:
            d()

    def loop(lo, hi, body):
        def wrapped(i, c):
            body(i)
            return c
        lax.fori_loop(lo, hi, wrapped, 0)

    def wait_all(ref, sem):
        pltpu.make_async_copy(ref, ref, sem).wait()

    def acc_cols(dst, part):
        for j in range(part.shape[1] // 128):
            dst[j * 8:(j + 1) * 8, :] += part[:, j * 128:(j + 1) * 128]

    loop(0, SKEW, lambda u: issue([partial(wo_copy, u, j) for j in range(8)]))
    small = [pltpu.make_async_copy(x_hbm, x_s, sem_w.at[4]),
             pltpu.make_async_copy(wr_hbm, wr_s, sem_w.at[5]),
             pltpu.make_async_copy(gw_hbm, gw_s, sem_w.at[6])]
    for c in small:
        c.start()
    loop(0, 28, lambda u: issue(pairs(partial(gate_up_copy, 0, u), partial(wo_copy, u + SKEW))))

    for c in small:
        c.wait()
    x4 = x_s[...].astype(F32)
    x8 = jnp.concatenate([x4, jnp.zeros_like(x4)], axis=0)
    for kb in range(KB):
        xb_s[kb] = x8[:, kb * 128:(kb + 1) * 128]
    gate = jax.nn.sigmoid(jnp.sum(x8 * gw_s[...].astype(F32).reshape(1, D), axis=-1, keepdims=True))
    rsel = jax.nn.sigmoid(jnp.sum(x8 * wr_s[...].astype(F32).reshape(1, D), axis=-1, keepdims=True))
    sc_s[0] = jnp.broadcast_to(gate, (8, 128))
    sc_s[1] = jnp.broadcast_to(rsel, (8, 128))
    q_s[...] = jnp.zeros_like(q_s)
    gu_s[...] = jnp.zeros_like(gu_s)
    o_s[...] = jnp.zeros_like(o_s)
    a_s[...] = jnp.zeros_like(a_s)
    y_s[...] = jnp.zeros_like(y_s)

    issue(pairs(partial(wq_copy, 0), partial(wo_copy, 31)))
    loop(1, 29, lambda u: issue(pairs(partial(wq_copy, u), partial(gate_up_copy, 1, u - 1))))
    loop(29, 32, lambda u: issue(pairs(partial(wq_copy, u), partial(wd_band_copy, 1, u - 29))))
    loop(0, 8 - SKEW, lambda u: issue(pairs(partial(wd_band_copy, 0, u), partial(wd_band_copy, 1, u + SKEW))))
    loop(8 - SKEW, 8, lambda u: issue(pairs(partial(wd_band_copy, 0, u), partial(kv_copy, 1, u - (8 - SKEW)))))

    def kv_pairs(t):
        return pairs(partial(kv_copy, 0, t), partial(kv_copy, 1, t + SKEW))

    loop(0, LK - KB // 2, lambda t: issue(kv_pairs(t)))
    wait_all(wq_s, sem_w.at[2])

    def q_proj(t):
        issue(kv_pairs(t))
        kb = (t - (LK - KB // 2)) * 2
        acc_cols(q_s, jnp.dot(xb_s[kb].astype(BF16), wq_s[kb], preferred_element_type=F32)
                 + jnp.dot(xb_s[kb + 1].astype(BF16), wq_s[kb + 1], preferred_element_type=F32))
    loop(LK - KB // 2, LK, q_proj)

    neg = jnp.full((8, 128), -jnp.inf, F32)
    zero = jnp.zeros((8, 128), F32)
    row = lax.broadcasted_iota(jnp.int32, (8, R), 0)

    def block_rows(ref, b):
        return ref.at[b // 4, pl.ds(pl.multiple_of((b % 4) * 128, 128), 128)]

    def wo_block(h):
        lhs = o_s[pl.ds(h, 8, stride=H), :].astype(BF16)
        return jnp.dot(lhs, block_rows(wo_s, h)[...], preferred_element_type=F32)

    def wd_block(b):
        lhs = h_s[pl.ds(pl.multiple_of(b * 8, 8), 8), :].astype(BF16)
        return jnp.dot(lhs, block_rows(wd_s, b)[...], preferred_element_type=F32)

    def finalize(g, l, acc):
        o_s[pl.ds(pl.multiple_of(g * 8, 8), 8), :] = acc / jnp.sum(l, axis=-1, keepdims=True)

    def step(t, carry, dmas):
        m, l, acc = carry
        g = t // NS
        ks, vs = slot(t, 0), slot(t, 1)
        wait_all(kv.at[ks], sem_kv.at[ks])
        wait_all(kv.at[vs], sem_kv.at[vs])
        first = t % NS == 0
        m = jnp.where(first, neg, m)
        l = jnp.where(first, zero, l)
        acc = jnp.where(first, zero, acc)
        q = q_s[pl.ds((g % 4) * 64 + g // 4, 8, stride=8), :].astype(BF16)
        s = None
        for j in range(HG):
            issue(dmas[j:j + 1])
            sj = lax.dot_general(q, kv[ks, j], (((1,), (1,)), ((), ())), preferred_element_type=F32)
            s = sj if s is None else jnp.where(row == j, sj, s)
        s = s * SCALE
        m_new = jnp.maximum(m, jnp.max(s, axis=-1, keepdims=True))
        alpha = jnp.exp(m - m_new)
        p = jnp.exp(s - m_new)
        l = l * alpha + p
        pv = None
        for j in range(HG):
            issue(dmas[HG + j:HG + j + 1])
            pj = jnp.where(row == j, p, 0.0).astype(BF16)
            d = jnp.dot(pj, kv[vs, j], preferred_element_type=F32)
            pv = d if pv is None else pv + d
        return m_new, l, acc * alpha + pv

    def main_step(t, cr):
        cr = step(t, cr, kv_pairs(t + LK))

        @pl.when(t % NS == NS - 1)
        def _():
            finalize(t // NS, cr[1], cr[2])

        @pl.when(t < 2 * KB)
        def _():
            acc_cols(gu_s.at[t % 2],
                     jnp.dot(xb_s[t // 2].astype(BF16), wgu_s[t % 2, t // 2], preferred_element_type=F32))

        @pl.when(t == 2 * KB)
        def _():
            gg = gu_s[0]
            h_s[...] = gg * jax.nn.sigmoid(gg) * gu_s[1]

        @pl.when(jnp.logical_and(t > 2 * KB, t <= 2 * KB + WD_END))
        def _():
            y_s[...] += wd_block(t - (2 * KB + 1))

        @pl.when(t >= WO_T0)
        def _():
            a_s[...] += wo_block(t - WO_T0)
        return cr

    wait_all(wo_s, sem_w.at[3])
    wait_all(wd_s.at[0:BANDS], sem_w.at[7])
    wait_all(wgu_s.at[0], sem_w.at[0])
    wait_all(wgu_s.at[1], sem_w.at[1])
    cr = lax.fori_loop(0, T - LV, main_step, (neg, zero, zero))

    def tail_step(it, cr):
        t = T - LV + it

        @pl.when(it < SKEW)
        def _():
            issue(pairs(partial(kv_copy, 0, t + LK), partial(wd_copy, WD_END + jnp.minimum(1 + 2 * it, 2 + it), 1)))

        @pl.when(jnp.logical_and(it >= SKEW, it < SKEW + 2))
        def _():
            issue(pairs(partial(wd_copy, WD_END + 2 * (it - SKEW), 0), partial(wd_copy, WD_END + 2 + it, 1)))

        @pl.when(it == SKEW + 2)
        def _():
            for j in range(4):
                wd_copy(FB - 1, 0, j)
                wd_copy(FB - 1, 1, 4 + j)
        return step(t, cr, [])
    cr = lax.fori_loop(0, LV, tail_step, cr)
    finalize(G - 1, cr[1], cr[2])
    a = a_s[...]
    for h in range(H - HG, H):
        a = a + wo_block(h)
    gate = sc_s[0]
    coef = (1.0 - gate) * sc_s[1]
    base = [gate * a[:, kb * 128:(kb + 1) * 128] + (1.0 - gate) * xb_s[kb] for kb in range(KB)]

    def down(b, acc):
        wait_all(block_rows(wd_s, b), sem_wd.at[b - WD_END])
        return acc + wd_block(b)
    y = lax.fori_loop(WD_END, FB, down, y_s[...])

    out = jnp.concatenate([base[kb] + coef * y[:, kb * 128:(kb + 1) * 128] for kb in range(KB)], axis=1)
    o_ref[...] = out[0:B].astype(o_ref.dtype)


@jax.jit
def pallas_gated_mix__mha_block_cached__moe_arch_mod__decode_kernel(
    A_x: jax.Array,
    A_k_cache: jax.Array,
    A_v_cache: jax.Array,
    A_wq: jax.Array,
    A_wo: jax.Array,
    B_x: jax.Array,
    B_w_r: jax.Array,
    B_w_gate: jax.Array,
    B_w_up: jax.Array,
    B_w_down: jax.Array,
    gate_w: jax.Array,
):
    del B_x
    out = pl.pallas_call(
        _kernel,
        out_shape=jax.ShapeDtypeStruct((B, D), BF16),
        in_specs=[pl.BlockSpec(memory_space=pl.ANY)] * 10,
        out_specs=pl.BlockSpec(memory_space=pltpu.VMEM),
        scratch_shapes=[
            pltpu.VMEM((NBK + NBV, HG, R, DH), BF16),
            pltpu.VMEM((8, 128, H * DH), BF16),
            pltpu.VMEM((8, 512, D), BF16),
            pltpu.VMEM((2, 8, 128, F), BF16),
            pltpu.VMEM((7, 512, D), BF16),
            pltpu.VMEM((B, D), BF16),
            pltpu.VMEM((D,), BF16),
            pltpu.VMEM((D,), BF16),
            pltpu.VMEM((KB, 8, 128), F32),
            pltpu.VMEM((H * 8 + 8, 128), F32),
            pltpu.VMEM((2 * B * H + H, 128), F32),
            pltpu.VMEM((2, FB * 8, 128), F32),
            pltpu.VMEM((FB * 8, 128), F32),
            pltpu.VMEM((2, 8, 128), F32),
            pltpu.VMEM((8, D), F32),
            pltpu.VMEM((8, D), F32),
            pltpu.SemaphoreType.DMA((NBK + NBV,)),
            pltpu.SemaphoreType.DMA((8,)),
            pltpu.SemaphoreType.DMA((FB - WD_END,)),
        ],
        compiler_params=pltpu.CompilerParams(**_PARAMS),
    )(A_x.reshape(B, D), A_k_cache.reshape(G, HG, S, DH), A_v_cache.reshape(G, HG, S, DH),
      A_wq.reshape(8, 128, H * DH), A_wo.reshape(8, 512, D), B_w_r,
      B_w_gate.reshape(8, 128, F), B_w_up.reshape(8, 128, F), B_w_down.reshape(7, 512, D), gate_w)
    return out.reshape(B, 1, D)
```
